```python
import os as _os
_os.environ.setdefault("JAX_PLATFORMS", "cpu")
import jax
import jax.numpy as jnp

def _softmax(x, axis=-1):
    return jax.nn.softmax(x, axis=axis)
def _gelu(x):
    return jax.nn.gelu(x, approximate=True)
def _silu(x):
    return jax.nn.silu(x)
def _sigmoid(x):
    return jax.nn.sigmoid(x)
def _layernorm(x, axis=-1, eps=1e-5):
    m = jnp.mean(x, axis=axis, keepdims=True)
    v = jnp.var(x, axis=axis, keepdims=True)
    return (x - m) / jnp.sqrt(v + eps)
def _scatter_add(tgt, idx, src, axis=0):
    return tgt.at[idx].add(src)
def _segment_sum(src, seg, n):
    return jax.ops.segment_sum(src, seg, n)
class _Rng:
    def __init__(self, key):
        self._k = key
    def _next(self):
        self._k, sub = jax.random.split(self._k)
        return sub
    def normal(self, shape):
        return jax.random.normal(self._next(), shape, dtype=jnp.bfloat16)
    def randint(self, lo, hi, shape):
        return jax.random.randint(self._next(), shape, lo, hi, dtype=jnp.int32)
    def uniform(self, shape, lo=0.0, hi=1.0):
        return jax.random.uniform(self._next(), shape, jnp.bfloat16, lo, hi)
    def permutation(self, n):
        return jax.random.permutation(self._next(), n)


kernel_name = 'interleave_layers__linear_kernel_hedgehog__dense_activation_silu__prompt'

def setup_inputs():
    _rng = _Rng(jax.random.key(int.from_bytes(__import__("os").urandom(4), "little")))
    _w = (lambda a: (lambda t: t.astype(jnp.bfloat16) if jnp.issubdtype(t.dtype, jnp.floating) else t)(jnp.asarray(a)))
    def _A_setup():
        B, S, D, H = 1, 2048, 640, 32
        Dh = D // H
        return {
            "x": _w((lambda *s: _rng.normal(s) * 0.05)(B, S, D)),
            "wqkv": _w((lambda *s: _rng.normal(s) * 0.4)(D, 3 * D)),
            "w_phi": _w((lambda *s: _rng.normal(s) * 0.4)(H, Dh, Dh) * (Dh ** -0.5)),
            "wo": _w((lambda *s: _rng.normal(s) * 0.05)(D, D)),
        }
    _A_in = _A_setup()

    def _B_setup():
        B, S, D, F = 1, 2048, 640, 1728
        return {
            "x": _w((lambda *s: _rng.normal(s) * 0.05)(B, S, D)),
            "w1": _w((lambda *s: _rng.normal(s) * 1.6)(D, F) * (D ** -0.5)),
            "w2": _w((lambda *s: _rng.normal(s) * 1.6)(F, D) * (F ** -0.5)),
        }
    _B_in = _B_setup()

    return {
        "A_x": _A_in["x"],
        "A_wqkv": _A_in["wqkv"],
        "A_w_phi": _A_in["w_phi"],
        "A_wo": _A_in["wo"],
        "B_x": _B_in["x"],
        "B_w1": _B_in["w1"],
        "B_w2": _B_in["w2"],
    }

def reference(A_x, A_wqkv, A_w_phi, A_wo, B_x, B_w1, B_w2):
    def _A_ref(x, wqkv, w_phi, wo):
        B, S, D = x.shape
        H = 32; Dh = D // H
        qkv = (lambda x, *d: x.transpose(*d))((x @ wqkv).reshape(B, S, 3, H, Dh), 2, 0, 3, 1, 4)
        q, k, v = qkv[0], qkv[1], qkv[2]
        pq = jnp.einsum("bhsd,hdf->bhsf", q, w_phi)
        pk = jnp.einsum("bhsd,hdf->bhsf", k, w_phi)
        phi_q = jnp.concatenate([_softmax(pq, axis=-1), _softmax(-pq, axis=-1)], axis=-1)
        phi_k = jnp.concatenate([_softmax(pk, axis=-1), _softmax(-pk, axis=-1)], axis=-1)
        kv = jnp.einsum("bhsf,bhsd->bhfd", phi_k, v)
        z  = jnp.einsum("bhsf->bhf", phi_k)
        num = jnp.einsum("bhqf,bhfd->bhqd", phi_q, kv)
        den = jnp.einsum("bhqf,bhf->bhq", phi_q, z)[..., None] + 1e-6
        o = num / den
        return (lambda x, *d: x.transpose(*d))(o, 0, 2, 1, 3).reshape(B, S, D) @ wo

    def _B_ref(x, w1, w2):
        h = jnp.einsum("bsd,df->bsf", x, w1)
        h = _silu(h)
        out = jnp.einsum("bsf,fd->bsd", h, w2)
        return out

    x = A_x
    x = x + _A_ref(_layernorm(x, axis=-1), A_wqkv, A_w_phi, A_wo)
    x = x + _B_ref(_layernorm(x, axis=-1), B_w1, B_w2)
    x = x + _A_ref(_layernorm(x, axis=-1), A_wqkv, A_w_phi, A_wo)
    x = x + _B_ref(_layernorm(x, axis=-1), B_w1, B_w2)
    return x
```

```python
import functools
import jax
import jax.numpy as jnp
import numpy as np
from jax import lax
from jax.experimental import pallas as pl
from jax.experimental.pallas import tpu as pltpu

S, D, H, DH, F = 2048, 640, 32, 20, 1728
bf, f32, i32 = jnp.bfloat16, jnp.float32, jnp.int32
NT_DIMS = (((1,), (1,)), ((), ()))
LOG2E = 1.4426950408889634


def _iota(shape, dim):
    return lax.broadcasted_iota(i32, shape, dim)


def _mm(a, b):
    return jnp.dot(a, b, preferred_element_type=f32)


def _mm_nt(a, b):
    return lax.dot_general(a, b, NT_DIMS, preferred_element_type=f32)


def _ln_t(x, scale=1.0):
    m = jnp.sum(x, axis=0, keepdims=True) * (1.0 / D)
    xc = x - m
    v = jnp.sum(xc * xc, axis=0, keepdims=True) * (1.0 / D)
    r = lax.rsqrt(v + 1e-5)
    if scale != 1.0:
        r = r * scale
    return (xc * r).astype(bf)


def make(T=512, FC=F, HG=2):
    G = H // HG
    GR = HG * DH
    NV = GR // 8

    def red(x3, op):
        r = x3[0]
        for j in range(1, NV):
            r = op(r, x3[j])
        sft = HG
        while sft < 8:
            r = op(r, pltpu.roll(r, sft, 0))
            sft *= 2
        return r

    def _dual_exp(p, T):
        p3 = p.reshape(NV, 8, T)
        mx = red(p3, jnp.maximum)
        mn = red(p3, jnp.minimum)
        ep = jnp.exp2(p3 - mx[None])
        en = jnp.exp2(mn[None] - p3)
        return ep, en, red(ep, jnp.add), red(en, jnp.add)

    NTL = S // T
    LB = T // 128
    fchunks = [(s, min(F, s + FC)) for s in range(0, F, FC)]

    def kern(x_hbm, wqkv_hbm, wphi_hbm, wo_hbm, w1t_hbm, w2_hbm, o_hbm,
             xin, wqkv, wphi, wo, w2, w1t, wqT, wkvT, woT, w2T,
             X, XN, kvacc, zacc, kvm, zb, ostage, sems):
        def xcopy(i):
            return pltpu.make_async_copy(x_hbm.at[0, pl.ds(i * T, T), :], xin.at[i], sems.at[6 + i])
        c_phi = pltpu.make_async_copy(wphi_hbm, wphi, sems.at[0])
        c_kv = pltpu.make_async_copy(wqkv_hbm.at[:, pl.ds(D, 2 * D)], wqkv.at[:, pl.ds(D, 2 * D)], sems.at[1])
        c_q = pltpu.make_async_copy(wqkv_hbm.at[:, pl.ds(0, D)], wqkv.at[:, pl.ds(0, D)], sems.at[2])
        c_o = pltpu.make_async_copy(wo_hbm, wo, sems.at[3])
        c_w2 = pltpu.make_async_copy(w2_hbm, w2, sems.at[4])
        c_w1 = pltpu.make_async_copy(w1t_hbm, w1t, sems.at[5])
        c_phi.start(); c_kv.start(); xcopy(0).start()
        for i in range(1, NTL):
            xcopy(i).start()
        c_q.start(); c_o.start(); c_w2.start(); c_w1.start()

        c_phi.wait()
        wcat = jnp.concatenate([wphi[d].astype(f32) for d in range(DH)], axis=1)
        r_ = _iota((D, D), 0); c_ = _iota((D, D), 1)
        E = ((r_ % H) * DH + r_ // H == c_).astype(bf)
        Gm = _mm(wcat.astype(bf), E)

        SG = 4
        rr = _iota((160, 32), 0)
        onehot = ((rr % GR) // HG == _iota((160, 32), 1)).astype(bf)
        Gp = jnp.concatenate([Gm, jnp.zeros((32 - DH, D), f32)], axis=0).astype(bf)

        def bd(g):
            lo = 128 * (g * 160 // 128)
            rows = _mm(onehot, Gp[:, lo:lo + 256])
            r2 = _iota((160, 256), 0)
            head = 8 * g + (r2 // GR) * HG + r2 % HG
            own = (_iota((160, 256), 1) + lo) // DH == head
            return lo, jnp.where(own, rows, 0.0).astype(bf)
        bds = [bd(g) for g in range(SG)]

        def fold(dst, col0):
            for g in range(SG):
                lo, b = bds[g]
                w = _mm_nt(b, wqkv[:, col0 + lo: col0 + lo + 256])
                dst[g * 160:(g + 1) * 160, :] = (w * LOG2E).astype(bf)

        c_kv.wait()
        fold(wkvT, D)
        wkvT[D:2 * D, :] = wqkv[:, 2 * D:3 * D].T

        def kv_reset():
            kvacc[...] = jnp.zeros(kvacc.shape, f32)
            zacc[...] = jnp.zeros(zacc.shape, f32)

        def kv_part(i, x):
            xn = _ln_t(x)
            XN[i] = xn
            pv = _mm(wkvT[...], xn)
            for g in range(G):
                ep, en, sp, sn = _dual_exp(pv[g * GR:(g + 1) * GR], T)
                php = (ep * (1.0 / sp)[None]).reshape(GR, T)
                phn = (en * (1.0 / sn)[None]).reshape(GR, T)
                ph = jnp.concatenate([php, phn], axis=0)
                zs = ph[:, 0:128]
                for l in range(1, LB):
                    zs = zs + ph[:, l * 128:(l + 1) * 128]
                zacc[g] += zs
                v = pv[D + g * GR: D + (g + 1) * GR].astype(bf)
                kvacc[g] += _mm_nt(v, ph.astype(bf))

        def kv_finish():
            keep = _iota((GR, 2 * GR), 0) // DH == _iota((GR, 2 * GR), 1) % HG
            for g in range(G):
                kvm[g] = jnp.where(keep, kvacc[g], 0.0).astype(bf)
                zb[g] = jnp.broadcast_to(jnp.sum(zacc[g], axis=1, keepdims=True), (2 * GR, 128))

        def q_part(i):
            xn = XN[i]
            pq = _mm(wqT[...], xn)
            outs = []
            for g in range(G):
                ep, en, sp, sn = _dual_exp(pq[g * GR:(g + 1) * GR], T)
                z = zb[g]
                z = jnp.concatenate([z] * LB, axis=1) if LB > 1 else z
                zp = z[0:GR].reshape(NV, 8, T); zn = z[GR:2 * GR].reshape(NV, 8, T)
                dp = red(ep * zp, jnp.add); dn = red(en * zn, jnp.add)
                isp = 1.0 / sp; isn = 1.0 / sn
                iden = 1.0 / (dp * isp + dn * isn + 1e-6)
                php = (ep * (isp * iden)[None]).reshape(GR, T)
                phn = (en * (isn * iden)[None]).reshape(GR, T)
                ph = jnp.concatenate([php, phn], axis=0).astype(bf)
                outs.append(_mm(kvm[g], ph))
            o = jnp.concatenate(outs, axis=0).astype(bf)
            return X[i] + _mm(woT[...], o)

        def ffn(x):
            xn = _ln_t(x, 0.5)
            acc = x
            for (s, e) in fchunks:
                hh = _mm(w1t[s:e, :], xn)
                a = (hh + hh * jnp.tanh(hh)).astype(bf)
                acc = acc + _mm(w2T[:, s:e], a)
            return acc

        def ocopy(i):
            return pltpu.make_async_copy(ostage.at[i], o_hbm.at[0, pl.ds(i * T, T), :], sems.at[6 + i])

        kv_reset()

        @pl.loop(0, 3 * NTL)
        def _(it):
            ph = it // NTL
            i = it % NTL

            @pl.when(it == NTL)
            def _():
                c_q.wait(); fold(wqT, 0)
                c_o.wait(); woT[...] = wo[...].T
                c_w2.wait(); w2T[...] = w2[...].T
                c_w1.wait()

            @pl.when(jnp.logical_and(i == 0, ph > 0))
            def _():
                kv_finish(); kv_reset()

            @pl.when(ph == 0)
            def _():
                xcopy(i).wait()
                X[i] = xin[i].T.astype(f32)

            @pl.when(ph > 0)
            def _():
                X[i] = ffn(q_part(i))

            @pl.when(ph < 2)
            def _():
                kv_part(i, X[i])

            @pl.when(ph == 2)
            def _():
                ostage[i] = X[i].astype(bf).T
                ocopy(i).start()

        for i in range(NTL):
            ocopy(i).wait()

    @jax.jit
    def pallas_interleave_layers__linear_kernel_hedgehog__dense_activation_silu__prompt_kernel(A_x, A_wqkv, A_w_phi, A_wo, B_x, B_w1, B_w2):
        hbm = pl.BlockSpec(memory_space=pltpu.HBM)
        return pl.pallas_call(
            kern,
            in_specs=[hbm] * 6,
            out_specs=hbm,
            out_shape=jax.ShapeDtypeStruct((1, S, D), bf),
            scratch_shapes=[
                pltpu.VMEM((NTL, T, D), bf),
                pltpu.VMEM((D, 3 * D), bf),
                pltpu.VMEM((DH, DH, H), bf),
                pltpu.VMEM((D, D), bf),
                pltpu.VMEM((F, D), bf),
                pltpu.VMEM((F, D), bf),
                pltpu.VMEM((D, D), bf),
                pltpu.VMEM((2 * D, D), bf),
                pltpu.VMEM((D, D), bf),
                pltpu.VMEM((D, F), bf),
                pltpu.VMEM((NTL, D, T), f32),
                pltpu.VMEM((NTL, D, T), bf),
                pltpu.VMEM((G, GR, 2 * GR), f32),
                pltpu.VMEM((G, 2 * GR, 128), f32),
                pltpu.VMEM((G, GR, 2 * GR), bf),
                pltpu.VMEM((G, 2 * GR, 128), f32),
                pltpu.VMEM((NTL, T, D), bf),
                pltpu.SemaphoreType.DMA((6 + NTL,)),
            ],
            compiler_params=pltpu.CompilerParams(vmem_limit_bytes=100 * 1024 * 1024),
        )(A_x, A_wqkv, A_w_phi.transpose(1, 2, 0), A_wo, B_w1.T, B_w2)
    return pallas_interleave_layers__linear_kernel_hedgehog__dense_activation_silu__prompt_kernel


pallas_interleave_layers__linear_kernel_hedgehog__dense_activation_silu__prompt_kernel = make(T=512, HG=2)
```

```python
import jax
import jax.numpy as jnp
from jax import lax
from jax.experimental import pallas as pl
from jax.experimental.pallas import tpu as pltpu

S, D, H, DH, F = 2048, 640, 32, 20, 1728
T = 512
NTL = S // T
HG = 2
G = H // HG
GR = HG * DH
GA = GR + 8
NV = GR // 8
NK = D // 128
bf, f32, i32 = jnp.bfloat16, jnp.float32, jnp.int32
NT_DIMS = (((1,), (1,)), ((), ()))
LOG2E = 1.4426950408889634


def _iota(shape, dim):
    return lax.broadcasted_iota(i32, shape, dim)


def _mm(a, b):
    return jnp.dot(a, b, preferred_element_type=f32)


def _mm_nt(a, b):
    return lax.dot_general(a, b, NT_DIMS, preferred_element_type=f32)


def _ln_t(x, scale=1.0):
    m = jnp.sum(x, axis=0, keepdims=True) * (1.0 / D)
    xc = x - m
    v = jnp.sum(xc * xc, axis=0, keepdims=True) * (1.0 / D)
    r = lax.rsqrt(v + 1e-5)
    if scale != 1.0:
        r = r * scale
    return (xc * r).astype(bf)


def _head_reduce(x3, op):
    r = x3[0]
    for j in range(1, NV):
        r = op(r, x3[j])
    sft = HG
    while sft < 8:
        r = op(r, pltpu.roll(r, sft, 0))
        sft *= 2
    return r


def _feature_map(p):
    p3 = p.reshape(NV, 8, T)
    mx = _head_reduce(p3, jnp.maximum)
    mn = _head_reduce(p3, jnp.minimum)
    ep = jnp.exp2(p3 - mx[None])
    en = jnp.exp2(mn[None] - p3)
    sp = _head_reduce(ep, jnp.add)
    sn = _head_reduce(en, jnp.add)
    php = (ep * (1.0 / sp)[None]).reshape(GR, T)
    phn = (en * (1.0 / sn)[None]).reshape(GR, T)
    return jnp.concatenate([php, phn], axis=0).astype(bf)


def _kernel(x_hbm, wqkv_hbm, wphi_hbm, wo_hbm, w1t_hbm, w2_hbm, o_hbm,
         xin, wqkv, wphi, wo, w2, w1t, wqT, wkvT, woT, w2T,
         X, XN, kvacc, kvm, ostage, sems):
    def xcopy(i):
        return pltpu.make_async_copy(x_hbm.at[0, pl.ds(i * T, T), :], xin.at[i], sems.at[6 + i])
    c_phi = pltpu.make_async_copy(wphi_hbm, wphi, sems.at[0])
    c_k = pltpu.make_async_copy(wqkv_hbm.at[:, pl.ds(D, D)], wqkv.at[:, pl.ds(D, D)], sems.at[1])
    c_v = pltpu.make_async_copy(wqkv_hbm.at[:, pl.ds(2 * D, D)], wqkv.at[:, pl.ds(2 * D, D)], sems.at[6 + NTL])
    c_q = pltpu.make_async_copy(wqkv_hbm.at[:, pl.ds(0, D)], wqkv.at[:, pl.ds(0, D)], sems.at[2])
    c_o = pltpu.make_async_copy(wo_hbm, wo, sems.at[3])
    c_w2 = pltpu.make_async_copy(w2_hbm, w2, sems.at[4])
    c_w1 = pltpu.make_async_copy(w1t_hbm, w1t, sems.at[5])
    c_phi.start()
    c_k.start(); xcopy(0).start(); c_v.start(); xcopy(1).start()
    for i in range(2, NTL):
        xcopy(i).start()
    c_q.start(); c_o.start(); c_w2.start(); c_w1.start()

    c_phi.wait()
    wcat = jnp.concatenate([wphi[d].astype(f32) for d in range(DH)], axis=1)
    r_ = _iota((D, D), 0); c_ = _iota((D, D), 1)
    E = ((r_ % H) * DH + r_ // H == c_).astype(bf)
    Gm = _mm(wcat.astype(bf), E)

    rr = _iota((160, 32), 0)
    onehot = ((rr % GR) // HG == _iota((160, 32), 1)).astype(bf)
    Gp = jnp.concatenate([Gm, jnp.zeros((32 - DH, D), f32)], axis=0).astype(bf)

    def bd(j):
        r0 = GR * (128 * j // GR)
        rows = _mm(onehot, Gp[:, 128 * j:128 * (j + 1)])
        r2 = _iota((160, 128), 0)
        head = ((r2 + r0) // GR) * HG + r2 % HG
        own = (_iota((160, 128), 1) + 128 * j) // DH == head
        return jnp.where(own, rows, 0.0).astype(bf)
    bds = [bd(j) for j in range(NK)]

    def fold(dst, col0):
        res = [_mm_nt(bds[j], wqkv[:, col0 + 128 * j: col0 + 128 * (j + 1)]) for j in range(NK)]
        parts = []
        for j in range(NK):
            top = res[j][0:GR] if j == 0 else res[j][0:GR] + res[j - 1][3 * GR:4 * GR]
            nrow = 4 * GR if j == NK - 1 else 3 * GR
            parts += [top, res[j][GR:nrow]]
        dst[0:D, :] = (jnp.concatenate(parts, axis=0) * LOG2E).astype(bf)

    eye = (_iota((128, 128), 0) == _iota((128, 128), 1)).astype(bf)

    def transpose_into(dst, row0, src, col0, ncols, nx):
        if nx > 0:
            dst[row0:row0 + 128 * nx, :] = src[:, col0:col0 + 128 * nx].T
        for j in range(nx, ncols // 128):
            blk = src[:, col0 + 128 * j: col0 + 128 * (j + 1)]
            dst[row0 + 128 * j: row0 + 128 * (j + 1), :] = _mm_nt(eye, blk).astype(bf)

    def load_x(i):
        x = xin[i].T.astype(f32)
        X[i] = x
        XN[i] = _ln_t(x)

    c_k.wait()
    fold(wkvT, D)
    xcopy(0).wait()
    load_x(0)
    c_v.wait()
    transpose_into(wkvT, D, wqkv, 2 * D, D, 3)

    def kv_reset():
        kvacc[...] = jnp.zeros(kvacc.shape, f32)

    def kv_part(i):
        xn = XN[i]
        pv = _mm(wkvT[...], xn)
        ones = jnp.ones((8, T), f32)
        for g in range(G):
            ph = _feature_map(pv[g * GR:(g + 1) * GR])
            v = jnp.concatenate([pv[D + g * GR: D + (g + 1) * GR], ones], axis=0).astype(bf)
            kvacc[g] += _mm_nt(v, ph)

    def kv_finish():
        r = _iota((GA, 2 * GR), 0)
        head = jnp.where(r < GR, r // DH, (r - GR) // 4)
        keep = head == _iota((GA, 2 * GR), 1) % HG
        for g in range(G):
            kvm[g] = jnp.where(keep, kvacc[g], 0.0).astype(bf)

    def q_part(i):
        xn = XN[i]
        pq = _mm(wqT[...], xn)
        low = _iota((8, T), 0) < 4
        outs = []
        for g in range(G):
            ph = _feature_map(pq[g * GR:(g + 1) * GR])
            res = _mm(kvm[g], ph)
            inv = 1.0 / (res[GR:GA] + 1e-6)
            swp = pltpu.roll(inv, 4, 0)
            a0 = jnp.where(low, inv, swp)
            a1 = jnp.where(low, swp, inv)
            outs += [res[0:8] * a0, res[8:16] * a0, res[16:24] * inv, res[24:32] * a1, res[32:40] * a1]
        o = jnp.concatenate(outs, axis=0).astype(bf)
        return X[i] + _mm(woT[...], o)

    def ffn(x):
        xn = _ln_t(x, 0.5)
        hh = _mm(w1t[...], xn)
        a = (hh + hh * jnp.tanh(hh)).astype(bf)
        return x + _mm(w2T[...], a)

    def ocopy(i):
        return pltpu.make_async_copy(ostage.at[i], o_hbm.at[0, pl.ds(i * T, T), :], sems.at[6 + i])

    kv_reset()

    @pl.loop(0, NTL)
    def _(i):
        nxt = jnp.minimum(i + 1, NTL - 1)

        @pl.when(i + 1 < NTL)
        def _():
            xcopy(nxt).wait()

        kv_part(i)
        load_x(nxt)

    c_q.wait(); c_o.wait(); c_w2.wait(); c_w1.wait()
    kv_finish(); kv_reset()
    fold(wqT, 0)
    transpose_into(woT, 0, wo, 0, D, 1)
    transpose_into(w2T, 0, w2, 0, D, 5)

    @pl.loop(0, 2 * NTL)
    def _(it):
        i = it % NTL
        x = ffn(q_part(i))
        X[i] = x
        XN[i] = _ln_t(x)
        ostage[i] = x.astype(bf).T

        @pl.when(it < NTL)
        def _():
            kv_part(i)

        @pl.when(it == NTL - 1)
        def _():
            kv_finish()

        @pl.when(it >= NTL)
        def _():
            ocopy(i).start()

    for i in range(NTL):
        ocopy(i).wait()

@jax.jit
def pallas_interleave_layers__linear_kernel_hedgehog__dense_activation_silu__prompt_kernel(A_x, A_wqkv, A_w_phi, A_wo, B_x, B_w1, B_w2):
    del B_x
    hbm = pl.BlockSpec(memory_space=pltpu.HBM)
    return pl.pallas_call(
        _kernel,
        in_specs=[hbm] * 6,
        out_specs=hbm,
        out_shape=jax.ShapeDtypeStruct((1, S, D), bf),
        scratch_shapes=[
            pltpu.VMEM((NTL, T, D), bf),
            pltpu.VMEM((D, 3 * D), bf),
            pltpu.VMEM((DH, DH, H), bf),
            pltpu.VMEM((D, D), bf),
            pltpu.VMEM((F, D), bf),
            pltpu.VMEM((F, D), bf),
            pltpu.VMEM((D, D), bf),
            pltpu.VMEM((2 * D, D), bf),
            pltpu.VMEM((D, D), bf),
            pltpu.VMEM((D, F), bf),
            pltpu.VMEM((NTL, D, T), f32),
            pltpu.VMEM((NTL, D, T), bf),
            pltpu.VMEM((G, GR + 8, 2 * GR), f32),
            pltpu.VMEM((G, GR + 8, 2 * GR), bf),
            pltpu.VMEM((NTL, T, D), bf),
            pltpu.SemaphoreType.DMA((7 + NTL,)),
        ],
        compiler_params=pltpu.CompilerParams(vmem_limit_bytes=100 * 1024 * 1024),
    )(A_x, A_wqkv, A_w_phi.transpose(1, 2, 0), A_wo, B_w1.T, B_w2)
```

```python
import jax
import jax.numpy as jnp
from jax import lax
from jax.experimental import pallas as pl
from jax.experimental.pallas import tpu as pltpu

S, D, H, DH, F = 2048, 640, 32, 20, 1728
T = 512
NTL = S // T
HG = 2
G = H // HG
GR = HG * DH
GA = GR + 8
NV = GR // 8
NK = D // 128
bf, f32, i32 = jnp.bfloat16, jnp.float32, jnp.int32
NT_DIMS = (((1,), (1,)), ((), ()))
LOG2E = 1.4426950408889634


def _iota(shape, dim):
    return lax.broadcasted_iota(i32, shape, dim)


def _mm(a, b):
    return jnp.dot(a, b, preferred_element_type=f32)


def _mm_nt(a, b):
    return lax.dot_general(a, b, NT_DIMS, preferred_element_type=f32)


def _ln_t(x, scale=1.0):
    m = jnp.sum(x, axis=0, keepdims=True) * (1.0 / D)
    xc = x - m
    v = jnp.sum(xc * xc, axis=0, keepdims=True) * (1.0 / D)
    r = lax.rsqrt(v + 1e-5)
    if scale != 1.0:
        r = r * scale
    return (xc * r).astype(bf)


def _head_reduce(x3, op):
    r = x3[0]
    for j in range(1, NV):
        r = op(r, x3[j])
    sft = HG
    while sft < 8:
        r = op(r, pltpu.roll(r, sft, 0))
        sft *= 2
    return r


def _feature_map(p):
    p3 = p.reshape(NV, 8, T)
    mx = _head_reduce(p3, jnp.maximum)
    mn = _head_reduce(p3, jnp.minimum)
    ep = jnp.exp2(p3 - mx[None])
    en = jnp.exp2(mn[None] - p3)
    sp = _head_reduce(ep, jnp.add)
    sn = _head_reduce(en, jnp.add)
    php = (ep * (1.0 / sp)[None]).reshape(GR, T)
    phn = (en * (1.0 / sn)[None]).reshape(GR, T)
    return jnp.concatenate([php, phn], axis=0).astype(bf)


def _kernel(x_hbm, wqkv_hbm, wphi_hbm, wo_hbm, w1t_hbm, w2_hbm, o_hbm,
         xin, wqkv, wphi, wo, w2, w1t, wqT, wkvT, woT, w2T,
         X, XN, kvacc, kvm, ostage, sems):
    def xcopy(i):
        return pltpu.make_async_copy(x_hbm.at[0, pl.ds(i * T, T), :], xin.at[i], sems.at[6 + i])
    c_phi = pltpu.make_async_copy(wphi_hbm, wphi, sems.at[0])
    c_k = pltpu.make_async_copy(wqkv_hbm.at[:, pl.ds(D, D)], wqkv.at[:, pl.ds(D, D)], sems.at[1])
    c_v = pltpu.make_async_copy(wqkv_hbm.at[:, pl.ds(2 * D, D)], wqkv.at[:, pl.ds(2 * D, D)], sems.at[6 + NTL])
    c_q = pltpu.make_async_copy(wqkv_hbm.at[:, pl.ds(0, D)], wqkv.at[:, pl.ds(0, D)], sems.at[2])
    c_o = pltpu.make_async_copy(wo_hbm, wo, sems.at[3])
    c_w2 = pltpu.make_async_copy(w2_hbm, w2, sems.at[4])
    c_w1 = pltpu.make_async_copy(w1t_hbm, w1t, sems.at[5])
    c_phi.start()
    c_k.start(); xcopy(0).start(); c_v.start(); xcopy(1).start()
    for i in range(2, NTL):
        xcopy(i).start()
    c_q.start(); c_o.start(); c_w2.start(); c_w1.start()

    c_phi.wait()
    wcat = jnp.concatenate([wphi[d].astype(f32) for d in range(DH)], axis=1)
    r_ = _iota((D, D), 0); c_ = _iota((D, D), 1)
    E = ((r_ % H) * DH + r_ // H == c_).astype(bf)
    Gm = _mm(wcat.astype(bf), E)

    rr = _iota((160, 32), 0)
    onehot = ((rr % GR) // HG == _iota((160, 32), 1)).astype(bf)
    Gp = jnp.concatenate([Gm, jnp.zeros((32 - DH, D), f32)], axis=0).astype(bf)

    def bd(j):
        r0 = GR * (128 * j // GR)
        rows = _mm(onehot, Gp[:, 128 * j:128 * (j + 1)])
        r2 = _iota((160, 128), 0)
        head = ((r2 + r0) // GR) * HG + r2 % HG
        own = (_iota((160, 128), 1) + 128 * j) // DH == head
        return jnp.where(own, rows, 0.0).astype(bf)
    bds = [bd(j) for j in range(NK)]

    def fold(dst, col0):
        res = [_mm_nt(bds[j], wqkv[:, col0 + 128 * j: col0 + 128 * (j + 1)]) for j in range(NK)]
        parts = []
        for j in range(NK):
            top = res[j][0:GR] if j == 0 else res[j][0:GR] + res[j - 1][3 * GR:4 * GR]
            nrow = 4 * GR if j == NK - 1 else 3 * GR
            parts += [top, res[j][GR:nrow]]
        dst[0:D, :] = (jnp.concatenate(parts, axis=0) * LOG2E).astype(bf)

    eye = (_iota((128, 128), 0) == _iota((128, 128), 1)).astype(bf)

    def transpose_into(dst, row0, src, col0, ncols, nx):
        if nx > 0:
            dst[row0:row0 + 128 * nx, :] = src[:, col0:col0 + 128 * nx].T
        for j in range(nx, ncols // 128):
            blk = src[:, col0 + 128 * j: col0 + 128 * (j + 1)]
            dst[row0 + 128 * j: row0 + 128 * (j + 1), :] = _mm_nt(eye, blk).astype(bf)

    def load_x(i):
        x = xin[i].T.astype(f32)
        X[i] = x
        XN[i] = _ln_t(x)

    c_k.wait()
    fold(wkvT, D)
    xcopy(0).wait()
    load_x(0)
    c_v.wait()
    transpose_into(wkvT, D, wqkv, 2 * D, D, 3)

    def kv_reset():
        kvacc[...] = jnp.zeros(kvacc.shape, f32)

    def kv_part(i):
        xn = XN[i]
        pv = _mm(wkvT[...], xn)
        ones = jnp.ones((8, T), f32)
        for g in range(G):
            ph = _feature_map(pv[g * GR:(g + 1) * GR])
            v = jnp.concatenate([pv[D + g * GR: D + (g + 1) * GR], ones], axis=0).astype(bf)
            kvacc[g] += _mm_nt(v, ph)

    def kv_finish():
        r = _iota((GA, 2 * GR), 0)
        head = jnp.where(r < GR, r // DH, (r - GR) // 4)
        keep = head == _iota((GA, 2 * GR), 1) % HG
        for g in range(G):
            kvm[g] = jnp.where(keep, kvacc[g], 0.0).astype(bf)

    def q_part(i):
        xn = XN[i]
        pq = _mm(wqT[...], xn)
        low = _iota((8, T), 0) < 4
        outs = []
        for g in range(G):
            ph = _feature_map(pq[g * GR:(g + 1) * GR])
            res = _mm(kvm[g], ph)
            inv = 1.0 / (res[GR:GA] + 1e-6)
            swp = pltpu.roll(inv, 4, 0)
            a0 = jnp.where(low, inv, swp)
            a1 = jnp.where(low, swp, inv)
            outs += [res[0:8] * a0, res[8:16] * a0, res[16:24] * inv, res[24:32] * a1, res[32:40] * a1]
        o = jnp.concatenate(outs, axis=0).astype(bf)
        return X[i] + _mm(woT[...], o)

    def ffn(x):
        xn = _ln_t(x, 0.5)
        hh = _mm(w1t[...], xn)
        a = (hh + hh * jnp.tanh(hh)).astype(bf)
        return x + _mm(w2T[...], a)

    def ocopy(i):
        return pltpu.make_async_copy(ostage.at[i], o_hbm.at[0, pl.ds(i * T, T), :], sems.at[6 + i])

    kv_reset()

    xcopy(1).wait()
    kv_part(0)
    load_x(1)
    for i in range(2, NTL):
        xcopy(i).wait()
    for i in range(1, NTL - 1):
        load_x(i + 1)
        kv_part(i)

    @pl.loop(-1, 2 * NTL)
    def _(it):
        i = (it + NTL) % NTL

        @pl.when(it >= 0)
        def _():
            x = ffn(q_part(i))
            X[i] = x
            XN[i] = _ln_t(x)
            ostage[i] = x.astype(bf).T

        @pl.when(it < NTL)
        def _():
            kv_part(i)

        @pl.when(it == -1)
        def _():
            c_q.wait(); c_o.wait(); c_w2.wait(); c_w1.wait()
            kv_finish(); kv_reset()
            fold(wqT, 0)
            transpose_into(woT, 0, wo, 0, D, 1)
            transpose_into(w2T, 0, w2, 0, D, 5)

        @pl.when(it == NTL - 1)
        def _():
            kv_finish()

        @pl.when(it >= NTL)
        def _():
            ocopy(i).start()

    for i in range(NTL):
        ocopy(i).wait()

@jax.jit
def pallas_interleave_layers__linear_kernel_hedgehog__dense_activation_silu__prompt_kernel(A_x, A_wqkv, A_w_phi, A_wo, B_x, B_w1, B_w2):
    del B_x
    hbm = pl.BlockSpec(memory_space=pltpu.HBM)
    return pl.pallas_call(
        _kernel,
        in_specs=[hbm] * 6,
        out_specs=hbm,
        out_shape=jax.ShapeDtypeStruct((1, S, D), bf),
        scratch_shapes=[
            pltpu.VMEM((NTL, T, D), bf),
            pltpu.VMEM((D, 3 * D), bf),
            pltpu.VMEM((DH, DH, H), bf),
            pltpu.VMEM((D, D), bf),
            pltpu.VMEM((F, D), bf),
            pltpu.VMEM((F, D), bf),
            pltpu.VMEM((D, D), bf),
            pltpu.VMEM((2 * D, D), bf),
            pltpu.VMEM((D, D), bf),
            pltpu.VMEM((D, F), bf),
            pltpu.VMEM((NTL, D, T), f32),
            pltpu.VMEM((NTL, D, T), bf),
            pltpu.VMEM((G, GR + 8, 2 * GR), f32),
            pltpu.VMEM((G, GR + 8, 2 * GR), bf),
            pltpu.VMEM((NTL, T, D), bf),
            pltpu.SemaphoreType.DMA((7 + NTL,)),
        ],
        compiler_params=pltpu.CompilerParams(vmem_limit_bytes=100 * 1024 * 1024),
    )(A_x, A_wqkv, A_w_phi.transpose(1, 2, 0), A_wo, B_w1.T, B_w2)
```
